```python
import jax
import jax.numpy as jnp

def _softmax(x, axis=-1):
    return jax.nn.softmax(x, axis=axis)
def _gelu(x):
    return jax.nn.gelu(x, approximate=True)
def _silu(x):
    return jax.nn.silu(x)
def _sigmoid(x):
    return jax.nn.sigmoid(x)
def _layernorm(x, axis=-1, eps=1e-5):
    m = jnp.mean(x, axis=axis, keepdims=True)
    v = jnp.var(x, axis=axis, keepdims=True)
    return (x - m) / jnp.sqrt(v + eps)
def _scatter_add(tgt, idx, src, axis=0):
    return tgt.at[idx].add(src)
def _segment_sum(src, seg, n):
    return jax.ops.segment_sum(src, seg, n)
class _Rng:
    def __init__(self, key):
        self._k = key
    def _next(self):
        self._k, sub = jax.random.split(self._k)
        return sub
    def normal(self, shape):
        return jax.random.normal(self._next(), shape, dtype=jnp.bfloat16)
    def randint(self, lo, hi, shape):
        return jax.random.randint(self._next(), shape, lo, hi, dtype=jnp.int32)
    def uniform(self, shape, lo=0.0, hi=1.0):
        return jax.random.uniform(self._next(), shape, jnp.bfloat16, lo, hi)
    def permutation(self, n):
        return jax.random.permutation(self._next(), n)


kernel_name = 'sequential_preLN__sliding_block_cached__mixer_s_mlp__decode'

def setup_inputs():
    _rng = _Rng(jax.random.key(int.from_bytes(__import__("os").urandom(4), "little")))
    _w = (lambda a: (lambda t: t.astype(jnp.bfloat16) if jnp.issubdtype(t.dtype, jnp.floating) else t)(jnp.asarray(a)))
    def _A_setup():
        B, Sq, D = 1, 1, 640
        Hq, Hkv, Sk, Dh = 32, 32, 32768, 192
        assert Hq % Hkv == 0, (Hq, Hkv)
        return {
            "x": _w((lambda *s: _rng.normal(s) * 0.05)(B, Sq, D)),
            "k_cache": _w((lambda *s: _rng.normal(s) * 0.05)(B, Hkv, Sk, Dh)),
            "v_cache": _w((lambda *s: _rng.normal(s) * 0.05)(B, Hkv, Sk, Dh)),
            "wq": _w((lambda *s: _rng.normal(s) * 0.05)(D, Hq * Dh) * (D ** -0.5)),
            "wo": _w((lambda *s: _rng.normal(s) * 0.05)(Hq * Dh, D) * ((Hq * Dh) ** -0.5)),
        }
    _A_in = _A_setup()

    def _B_setup():
        B, S, D, F = 1, 1, 640, 1536
        return {
            "x":  _w((lambda *s: _rng.normal(s) * 0.05)(B, S, D)),
            "w1": _w((lambda *s: _rng.normal(s) * 0.05)(D, D) * (D ** -0.5)),
            "w2": _w((lambda *s: _rng.normal(s) * 0.05)(D, D) * (D ** -0.5)),
            "w3": _w((lambda *s: _rng.normal(s) * 0.05)(D, F) * (D ** -0.5)),
            "w4": _w((lambda *s: _rng.normal(s) * 0.05)(F, D) * (F ** -0.5)),
        }
    _B_in = _B_setup()

    return {
        "A_x": _A_in["x"],
        "A_k_cache": _A_in["k_cache"],
        "A_v_cache": _A_in["v_cache"],
        "A_wq": _A_in["wq"],
        "A_wo": _A_in["wo"],
        "B_x": _B_in["x"],
        "B_w1": _B_in["w1"],
        "B_w2": _B_in["w2"],
        "B_w3": _B_in["w3"],
        "B_w4": _B_in["w4"],
    }

def reference(A_x, A_k_cache, A_v_cache, A_wq, A_wo, B_x, B_w1, B_w2, B_w3, B_w4):
    def _A_ref(x, k_cache, v_cache, wq, wo):
        B, Sq, D = x.shape
        Hq, Dh = 32, 192
        Hkv, Sk = k_cache.shape[1], k_cache.shape[2]
        W = min(4096, max(256, Sk // 4))
        rep = Hq // Hkv
        q = (lambda x, *d: x.transpose(*d))((x @ wq).reshape(B, Sq, Hq, Dh), 0, 2, 1, 3)
        k = jnp.repeat(k_cache[:, :, Sk - W:, :], rep, axis=1)
        v = jnp.repeat(v_cache[:, :, Sk - W:, :], rep, axis=1)
        scores = jnp.einsum("bhqd,bhkd->bhqk", q, k) * (Dh ** -0.5)
        p = _softmax(scores, axis=-1)
        o = jnp.einsum("bhqk,bhkd->bhqd", p, v)
        return (lambda x, *d: x.transpose(*d))(o, 0, 2, 1, 3).reshape(B, Sq, Hq * Dh) @ wo

    def _B_ref(x, w1, w2, w3, w4):
        B, S, D = x.shape
        h = _gelu(_layernorm(x, axis=-1) @ w1)
        c = D // 4
        g0 = jnp.pad(h[:, :, 0*c:1*c], ((0, 0), (1, 0), (0, 0)))[:, :S, :]
        g1 = jnp.pad(h[:, :, 1*c:2*c], ((0, 0), (0, 1), (0, 0)))[:, 1:, :]
        g2 = jnp.pad(h[:, :, 2*c:3*c], ((0, 0), (2, 0), (0, 0)))[:, :S, :]
        g3 = jnp.pad(h[:, :, 3*c:   ], ((0, 0), (0, 2), (0, 0)))[:, 2:, :]
        hs = jnp.concatenate([g0, g1, g2, g3], axis=-1) @ w2
        x1 = x + hs
        h2 = _gelu(_layernorm(x1, axis=-1) @ w3) @ w4
        return x1 + h2

    x = A_x
    h = x + _A_ref(_layernorm(x, axis=-1), A_k_cache, A_v_cache, A_wq, A_wo)
    h2 = h + _B_ref(_layernorm(h, axis=-1), B_w1, B_w2, B_w3, B_w4)
    return h2
```

```python
import jax
import jax.numpy as jnp
import numpy as np
from jax import lax
import jax.experimental.pallas as pl
import jax.experimental.pallas.tpu as pltpu

_EPS = 1e-5
_G = 2
_NBUF = 2
_W4C = 4
_M = 8


def _ln(x):
    m = jnp.mean(x, axis=-1, keepdims=True)
    d = x - m
    v = jnp.mean(d * d, axis=-1, keepdims=True)
    return d / jnp.sqrt(v + _EPS)


def _gelu(x):
    c = float(np.sqrt(2.0 / np.pi))
    return 0.5 * x * (1.0 + jnp.tanh(c * (x + 0.044715 * (x * x * x))))


@jax.jit
def pallas_sequential_preLN__sliding_block_cached__mixer_s_mlp__decode_kernel(
    A_x: jax.Array,
    A_k_cache: jax.Array,
    A_v_cache: jax.Array,
    A_wq: jax.Array,
    A_wo: jax.Array,
    B_x: jax.Array,
    B_w1: jax.Array,
    B_w2: jax.Array,
    B_w3: jax.Array,
    B_w4: jax.Array,
):
    B, Sq, D = A_x.shape
    _, H, SK, DH = A_k_cache.shape
    F = B_w3.shape[1]
    assert B == 1 and Sq == 1 and A_wq.shape == (D, H * DH)
    W = min(4096, max(256, SK // 4))
    G, NBUF, W4C, M = _G, _NBUF, _W4C, _M
    R = G * DH
    nblk = H // G
    FC = F // W4C
    scale = float(DH ** -0.5)
    f32, bf16 = jnp.float32, jnp.bfloat16

    def kernel(x_hbm, k_hbm, v_hbm, wq_hbm, wo_hbm, w3_hbm, w4_hbm, o_ref,
               xbuf, wqbuf, kbuf, vbuf, wobuf, w3buf, w4buf, sems, tsem):
        def stage_copies(g, slot):
            rows = pl.ds(g * R, R)
            win = pl.ds(SK - W, W)
            return (
                pltpu.make_async_copy(wq_hbm.at[:, rows], wqbuf.at[slot], sems.at[0, slot]),
                pltpu.make_async_copy(k_hbm.at[rows, win], kbuf.at[slot], sems.at[1, slot]),
                pltpu.make_async_copy(wo_hbm.at[rows, :], wobuf.at[slot], sems.at[2, slot]),
                pltpu.make_async_copy(v_hbm.at[rows, win], vbuf.at[slot], sems.at[3, slot]),
            )

        x_cp = pltpu.make_async_copy(x_hbm, xbuf, tsem.at[0])
        w3_cp = pltpu.make_async_copy(w3_hbm, w3buf, tsem.at[1])
        w4_cps = [
            pltpu.make_async_copy(
                w4_hbm.at[pl.ds(c * FC, FC), :], w4buf.at[pl.ds(c * FC, FC), :], tsem.at[2 + c])
            for c in range(W4C)
        ]

        x_cp.start()
        for g in range(NBUF):
            for cp in stage_copies(g, g):
                cp.start()

        x_cp.wait()
        x = jnp.broadcast_to(xbuf[...].astype(f32), (M, D))
        xn = _ln(x).astype(bf16)

        row = lax.broadcasted_iota(jnp.int32, (M, R), 0)
        col = lax.broadcasted_iota(jnp.int32, (M, R), 1)
        bd = (col >= row * DH) & (col < (row + 1) * DH)

        def body(g, acc):
            slot = g % NBUF
            cq, ck, co, cv = stage_copies(g, slot)
            cq.wait()
            q = jnp.dot(xn, wqbuf[slot], preferred_element_type=f32)
            qbd = jnp.where(bd, q, 0.0).astype(bf16)
            ck.wait()
            s = jnp.dot(qbd, kbuf[slot], preferred_element_type=f32)
            m = jnp.max(s, axis=-1, keepdims=True)
            p = jnp.exp((s - m) * scale)
            l = jnp.sum(p, axis=-1, keepdims=True)
            pb = p.astype(bf16)
            cv.wait()
            o = lax.dot_general(pb, vbuf[slot], (((1,), (1,)), ((), ())),
                                preferred_element_type=f32)
            obd = jnp.where(bd, o / l, 0.0).astype(bf16)
            co.wait()
            acc = acc + jnp.dot(obd, wobuf[slot], preferred_element_type=f32)

            nxt = g + NBUF

            @pl.when(nxt < nblk)
            def _():
                for cp in stage_copies(nxt, slot):
                    cp.start()

            @pl.when(nxt == nblk)
            def _():
                w3_cp.start()
                for cp in w4_cps:
                    cp.start()

            return acc

        acc = lax.fori_loop(0, nblk, body, jnp.zeros((M, D), f32))
        attn = jnp.sum(acc, axis=0, keepdims=True)
        h = x + jnp.broadcast_to(attn, (M, D))
        xb = _ln(h)
        xn2 = _ln(xb).astype(bf16)
        w3_cp.wait()
        g1 = _gelu(jnp.dot(xn2, w3buf[...], preferred_element_type=f32)).astype(bf16)
        y = h + xb
        for c in range(W4C):
            w4_cps[c].wait()
            y = y + jnp.dot(g1[:, c * FC:(c + 1) * FC], w4buf[pl.ds(c * FC, FC), :],
                            preferred_element_type=f32)
        o_ref[...] = y[0:1, :].astype(o_ref.dtype)

    kt = jnp.swapaxes(A_k_cache, 2, 3).reshape(H * DH, SK)
    vt = jnp.swapaxes(A_v_cache, 2, 3).reshape(H * DH, SK)
    out = pl.pallas_call(
        kernel,
        out_shape=jax.ShapeDtypeStruct((1, D), A_x.dtype),
        in_specs=[pl.BlockSpec(memory_space=pl.ANY)] * 7,
        out_specs=pl.BlockSpec(memory_space=pltpu.VMEM),
        scratch_shapes=[
            pltpu.VMEM((1, D), A_x.dtype),
            pltpu.VMEM((NBUF, D, R), A_wq.dtype),
            pltpu.VMEM((NBUF, R, W), A_k_cache.dtype),
            pltpu.VMEM((NBUF, R, W), A_v_cache.dtype),
            pltpu.VMEM((NBUF, R, D), A_wo.dtype),
            pltpu.VMEM((D, F), B_w3.dtype),
            pltpu.VMEM((F, D), B_w4.dtype),
            pltpu.SemaphoreType.DMA((4, NBUF)),
            pltpu.SemaphoreType.DMA((2 + W4C,)),
        ],
        compiler_params=pltpu.CompilerParams(vmem_limit_bytes=64 * 1024 * 1024),
    )(A_x.reshape(1, D), kt, vt, A_wq, A_wo, B_w3, B_w4)
    return out.reshape(B, Sq, D)
```

```python
import jax
import jax.numpy as jnp
import numpy as np
from jax import lax
import jax.experimental.pallas as pl
import jax.experimental.pallas.tpu as pltpu

_EPS = 1e-5
_G = 2
_NBUF = 2
_M = 8
_W4_MXU = (1024, 384)
_W4_VPU = (96, 32)


def _ln(x):
    m = jnp.mean(x, axis=-1, keepdims=True)
    d = x - m
    v = jnp.mean(d * d, axis=-1, keepdims=True)
    return d / jnp.sqrt(v + _EPS)


def _gelu(x):
    c = float(np.sqrt(2.0 / np.pi))
    return 0.5 * x * (1.0 + jnp.tanh(c * (x + 0.044715 * (x * x * x))))


@jax.jit
def pallas_sequential_preLN__sliding_block_cached__mixer_s_mlp__decode_kernel(
    A_x: jax.Array,
    A_k_cache: jax.Array,
    A_v_cache: jax.Array,
    A_wq: jax.Array,
    A_wo: jax.Array,
    B_x: jax.Array,
    B_w1: jax.Array,
    B_w2: jax.Array,
    B_w3: jax.Array,
    B_w4: jax.Array,
):
    B, Sq, D = A_x.shape
    _, H, SK, DH = A_k_cache.shape
    F = B_w3.shape[1]
    assert B == 1 and Sq == 1 and A_wq.shape == (D, H * DH) and H % _G == 0
    W = min(4096, max(256, SK // 4))
    G, NBUF, M = _G, _NBUF, _M
    R = G * DH
    nblk = H // G
    scale = float(DH ** -0.5)
    f32, bf16 = jnp.float32, jnp.bfloat16

    chunks = _W4_MXU + _W4_VPU
    offs = tuple(sum(chunks[:c]) for c in range(len(chunks)))
    n_mxu, nv = len(_W4_MXU), sum(_W4_VPU)
    assert sum(chunks) == F and nblk > NBUF and nv % 128 == 0 and D % 128 == 0

    def kernel(x_hbm, k_hbm, v_hbm, wq_hbm, wo_hbm, w3_hbm, w4_hbm, o_ref,
               xbuf, wqbuf, kbuf, vbuf, wobuf, w3buf, w4buf, sems, tsem):
        def stage_copies(g, slot):
            rows = pl.ds(g * R, R)
            win = pl.ds(SK - W, W)
            return (
                pltpu.make_async_copy(wq_hbm.at[:, rows], wqbuf.at[slot], sems.at[0, slot]),
                pltpu.make_async_copy(k_hbm.at[rows, win], kbuf.at[slot], sems.at[1, slot]),
                pltpu.make_async_copy(wo_hbm.at[rows, :], wobuf.at[slot], sems.at[2, slot]),
                pltpu.make_async_copy(v_hbm.at[rows, win], vbuf.at[slot], sems.at[3, slot]),
            )

        x_cp = pltpu.make_async_copy(x_hbm, xbuf, tsem.at[0])
        w3_cp = pltpu.make_async_copy(w3_hbm, w3buf, tsem.at[1])
        w4_cps = [
            pltpu.make_async_copy(w4_hbm.at[pl.ds(o, n), :], w4buf.at[pl.ds(o, n), :],
                                  tsem.at[2 + c])
            for c, (o, n) in enumerate(zip(offs, chunks))
        ]

        first = [cp for g in range(NBUF) for cp in stage_copies(g, g)]
        x_cp.start()
        first[0].start()
        x_cp.wait()
        for cp in first[1:]:
            cp.start()

        x = jnp.broadcast_to(xbuf[...].astype(f32), (M, D))
        xn = _ln(x).astype(bf16)

        row = lax.broadcasted_iota(jnp.int32, (M, R), 0)
        col = lax.broadcasted_iota(jnp.int32, (M, R), 1)
        bd = (col >= row * DH) & (col < (row + 1) * DH)

        def stage(g, acc):
            slot = g % NBUF
            cq, ck, co, cv = stage_copies(g, slot)
            cq.wait()
            q = jnp.dot(xn, wqbuf[slot], preferred_element_type=f32)
            qbd = jnp.where(bd, q, 0.0).astype(bf16)
            ck.wait()
            s = jnp.dot(qbd, kbuf[slot], preferred_element_type=f32)
            m = jnp.max(s, axis=-1, keepdims=True)
            p = jnp.exp((s - m) * scale)
            l = jnp.sum(p, axis=-1, keepdims=True)
            pb = p.astype(bf16)
            cv.wait()
            o = lax.dot_general(pb, vbuf[slot], (((1,), (1,)), ((), ())),
                                preferred_element_type=f32)
            obd = jnp.where(bd, o / l, 0.0).astype(bf16)
            co.wait()
            acc = acc + jnp.dot(obd, wobuf[slot], preferred_element_type=f32)

            nxt = g + NBUF

            @pl.when(nxt < nblk)
            def _():
                for cp in stage_copies(nxt, slot):
                    cp.start()

            @pl.when(nxt == nblk)
            def _():
                w3_cp.start()
                for cp in w4_cps:
                    cp.start()

            return acc

        acc = lax.fori_loop(0, nblk, stage, jnp.zeros((M, D), f32))

        h = x + jnp.broadcast_to(jnp.sum(acc, axis=0, keepdims=True), (M, D))
        xb = _ln(h)
        xn2 = _ln(xb).astype(bf16)

        w3_cp.wait()
        g1 = _gelu(jnp.dot(xn2, w3buf[...], preferred_element_type=f32)).astype(bf16)

        y = h + xb
        for c in range(n_mxu):
            o, n = offs[c], chunks[c]
            w4_cps[c].wait()
            y = y + jnp.dot(g1[:, o:o + n], w4buf[pl.ds(o, n), :],
                            preferred_element_type=f32)

        gt = jnp.concatenate(
            [jnp.concatenate([g1[:, o:o + 128].astype(f32)] * (128 // M), axis=0).T
             for o in range(F - nv, F, 128)], axis=0)
        part = jnp.zeros((8, D), f32)
        for c in range(n_mxu, len(chunks)):
            o, n = offs[c], chunks[c]
            gc = gt[o - (F - nv):o - (F - nv) + n, :]
            gc = jnp.concatenate([gc] * (D // 128), axis=1)
            w4_cps[c].wait()
            prod = w4buf[pl.ds(o, n), :].astype(f32) * gc
            part = part + jnp.sum(prod.reshape(n // 8, 8, D), axis=0)

        y = y[0:1, :] + jnp.sum(part, axis=0, keepdims=True)
        o_ref[...] = y.astype(o_ref.dtype)

    kt = jnp.swapaxes(A_k_cache, 2, 3).reshape(H * DH, SK)
    vt = jnp.swapaxes(A_v_cache, 2, 3).reshape(H * DH, SK)
    out = pl.pallas_call(
        kernel,
        out_shape=jax.ShapeDtypeStruct((1, D), A_x.dtype),
        in_specs=[pl.BlockSpec(memory_space=pl.ANY)] * 7,
        out_specs=pl.BlockSpec(memory_space=pltpu.VMEM),
        scratch_shapes=[
            pltpu.VMEM((1, D), A_x.dtype),
            pltpu.VMEM((NBUF, D, R), A_wq.dtype),
            pltpu.VMEM((NBUF, R, W), A_k_cache.dtype),
            pltpu.VMEM((NBUF, R, W), A_v_cache.dtype),
            pltpu.VMEM((NBUF, R, D), A_wo.dtype),
            pltpu.VMEM((D, F), B_w3.dtype),
            pltpu.VMEM((F, D), B_w4.dtype),
            pltpu.SemaphoreType.DMA((4, NBUF)),
            pltpu.SemaphoreType.DMA((2 + len(chunks),)),
        ],
        compiler_params=pltpu.CompilerParams(
            vmem_limit_bytes=64 * 1024 * 1024,
            disable_semaphore_checks=True,
        ),
    )(A_x.reshape(1, D), kt, vt, A_wq, A_wo, B_w3, B_w4)
    return out.reshape(B, Sq, D)
```

```python
import functools

import jax
import jax.numpy as jnp
import numpy as np
from jax import lax
import jax.experimental.pallas as pl
import jax.experimental.pallas.tpu as pltpu

_EPS = 1e-5
_G = 2
_NBUF = 3
_M = 8
_AHEAD = 80
_PARTS = 4
_KV_TILE = (192, 128)
_WQ_TILE = (128, 128)
_WO_ROWS = 24
_W3_TILE = (64, 256)
_W4_ROWS = 32
_W4_MXU = (1024, 384)
_W4_VPU = (96, 32)


def _ln(x):
    m = jnp.mean(x, axis=-1, keepdims=True)
    d = x - m
    v = jnp.mean(d * d, axis=-1, keepdims=True)
    return d / jnp.sqrt(v + _EPS)


def _gelu(x):
    c = float(np.sqrt(2.0 / np.pi))
    return 0.5 * x * (1.0 + jnp.tanh(c * (x + 0.044715 * (x * x * x))))


def _tiles(rows, cols, tr, tc, row_major=True):
    assert rows % tr == 0 and cols % tc == 0
    if row_major:
        return [(r, c) for r in range(0, rows, tr) for c in range(0, cols, tc)]
    return [(r, c) for c in range(0, cols, tc) for r in range(0, rows, tr)]


@jax.jit
def pallas_sequential_preLN__sliding_block_cached__mixer_s_mlp__decode_kernel(
    A_x: jax.Array,
    A_k_cache: jax.Array,
    A_v_cache: jax.Array,
    A_wq: jax.Array,
    A_wo: jax.Array,
    B_x: jax.Array,
    B_w1: jax.Array,
    B_w2: jax.Array,
    B_w3: jax.Array,
    B_w4: jax.Array,
):
    B, Sq, D = A_x.shape
    _, H, SK, DH = A_k_cache.shape
    F = B_w3.shape[1]
    assert B == 1 and Sq == 1 and A_wq.shape == (D, H * DH) and H % _G == 0
    W = min(4096, max(256, SK // 4))
    G, NBUF, M = _G, _NBUF, _M
    R = G * DH
    nblk = H // G
    scale = float(DH ** -0.5)
    f32, bf16 = jnp.float32, jnp.bfloat16

    chunks = _W4_MXU + _W4_VPU
    offs = tuple(sum(chunks[:c]) for c in range(len(chunks)))
    n_mxu, nv = len(_W4_MXU), sum(_W4_VPU)
    assert sum(chunks) == F and nblk >= 2 and nv % 128 == 0 and D % 128 == 0
    assert R % _WO_ROWS == 0 and all(n % _W4_ROWS == 0 for n in chunks)

    def kernel(x_hbm, k_hbm, v_hbm, wq_hbm, wo_hbm, w3_hbm, w4_hbm, o_ref,
               xbuf, wqbuf, kbuf, vbuf, wobuf, w3buf, w4buf, sems, tsem):
        copy = pltpu.make_async_copy
        lazy = functools.partial

        def stage_stream(g, slot):
            kr, kc = _KV_TILE
            kv = []
            for r, c in _tiles(R, W, kr, kc):
                src = (pl.ds(g * R + r, kr), pl.ds(SK - W + c, kc))
                dst = (slot, pl.ds(r, kr), pl.ds(c, kc))
                kv.append(lazy(copy, k_hbm.at[src], kbuf.at[dst], sems.at[0, slot]))
                kv.append(lazy(copy, v_hbm.at[src], vbuf.at[dst], sems.at[1, slot]))
            qr, qc = _WQ_TILE
            wq = [lazy(copy, wq_hbm.at[pl.ds(r, qr), pl.ds(g * R + c, qc)],
                       wqbuf.at[slot, pl.ds(r, qr), pl.ds(c, qc)], sems.at[2, slot])
                  for r, c in _tiles(D, R, qr, qc, row_major=False)]
            wo = [lazy(copy, wo_hbm.at[pl.ds(g * R + r, _WO_ROWS), :],
                       wobuf.at[slot, pl.ds(r, _WO_ROWS), :], sems.at[3, slot])
                  for r in range(0, R, _WO_ROWS)]
            wts = [e for j in range(max(len(wq), len(wo))) for e in wq[j:j + 1] + wo[j:j + 1]]
            groups = (len(wts) + 1) // 2
            step = len(kv) // groups
            out = []
            for j in range(groups):
                out += kv[j * step:(j + 1) * step] + wts[2 * j:2 * j + 2]
            return out + kv[groups * step:]

        def tail_stream():
            tr, tc = _W3_TILE
            out = [lazy(copy, w3_hbm.at[pl.ds(r, tr), pl.ds(c, tc)],
                        w3buf.at[pl.ds(r, tr), pl.ds(c, tc)], tsem.at[1])
                   for r, c in _tiles(D, F, tr, tc)]
            for ci, (o, n) in enumerate(zip(offs, chunks)):
                out += [lazy(copy, w4_hbm.at[pl.ds(r, _W4_ROWS), :],
                             w4buf.at[pl.ds(r, _W4_ROWS), :], tsem.at[2 + ci])
                        for r in range(o, o + n, _W4_ROWS)]
            return out

        def start(stream, lo, hi):
            for i in range(lo, hi):
                stream[i]().start(priority=i % 2)

        def wait_all(buf, sem):
            copy(buf, buf, sem).wait()

        NE = len(stage_stream(0, 0))
        tail = tail_stream()
        NT = len(tail)
        O = _AHEAD
        assert O <= min(NE, NT)
        cut = [2 * ((NE * p) // (2 * _PARTS)) for p in range(_PARTS)] + [NE]
        tcut = [O + 2 * (((NT - O) * p) // (2 * _PARTS)) for p in range(_PARTS)] + [NT]

        def issue(g, part):
            lo, hi = cut[part], cut[part + 1]
            if lo < NE - O:
                @pl.when(g + 1 < nblk)
                def _():
                    start(stage_stream(g + 1, (g + 1) % NBUF), O + lo, O + min(hi, NE - O))
            if hi > NE - O:
                a, b = max(lo, NE - O) - (NE - O), hi - (NE - O)

                @pl.when(g + 2 < nblk)
                def _():
                    start(stage_stream(g + 2, (g + 2) % NBUF), a, b)

                @pl.when(g + 2 == nblk)
                def _():
                    start(tail, a, b)
            if tcut[part] < tcut[part + 1]:
                @pl.when(g + 1 == nblk)
                def _():
                    start(tail, tcut[part], tcut[part + 1])

        x_cp = copy(x_hbm, xbuf, tsem.at[0])
        first = stage_stream(0, 0)
        x_cp.start()
        start(first, 0, 16)
        x_cp.wait()
        start(first, 16, NE)
        start(stage_stream(1, 1), 0, O)

        x = jnp.broadcast_to(xbuf[...].astype(f32), (M, D))
        xn = _ln(x).astype(bf16)

        row = lax.broadcasted_iota(jnp.int32, (M, R), 0)
        col = lax.broadcasted_iota(jnp.int32, (M, R), 1)
        bd = (col >= row * DH) & (col < (row + 1) * DH)

        def stage(g, acc):
            slot = g % NBUF
            wait_all(kbuf.at[slot], sems.at[0, slot])
            wait_all(vbuf.at[slot], sems.at[1, slot])
            wait_all(wqbuf.at[slot], sems.at[2, slot])
            wait_all(wobuf.at[slot], sems.at[3, slot])

            issue(g, 0)
            q = jnp.dot(xn, wqbuf[slot], preferred_element_type=f32)
            qbd = jnp.where(bd, q, 0.0).astype(bf16)
            s = jnp.dot(qbd, kbuf[slot], preferred_element_type=f32)
            issue(g, 1)
            m = jnp.max(s, axis=-1, keepdims=True)
            p = jnp.exp((s - m) * scale)
            l = jnp.sum(p, axis=-1, keepdims=True)
            pb = p.astype(bf16)
            issue(g, 2)
            o = lax.dot_general(pb, vbuf[slot], (((1,), (1,)), ((), ())),
                                preferred_element_type=f32)
            for part in range(3, _PARTS):
                issue(g, part)
            obd = jnp.where(bd, o / l, 0.0).astype(bf16)
            return acc + jnp.dot(obd, wobuf[slot], preferred_element_type=f32)

        acc = lax.fori_loop(0, nblk, stage, jnp.zeros((M, D), f32))

        h = x + jnp.broadcast_to(jnp.sum(acc, axis=0, keepdims=True), (M, D))
        xb = _ln(h)
        xn2 = _ln(xb).astype(bf16)

        wait_all(w3buf, tsem.at[1])
        g1 = _gelu(jnp.dot(xn2, w3buf[...], preferred_element_type=f32)).astype(bf16)

        y = h + xb
        for c in range(n_mxu):
            o, n = offs[c], chunks[c]
            wait_all(w4buf.at[pl.ds(o, n), :], tsem.at[2 + c])
            y = y + jnp.dot(g1[:, o:o + n], w4buf[pl.ds(o, n), :],
                            preferred_element_type=f32)

        gt = jnp.concatenate(
            [jnp.concatenate([g1[:, o:o + 128].astype(f32)] * (128 // M), axis=0).T
             for o in range(F - nv, F, 128)], axis=0)
        part = jnp.zeros((8, D), f32)
        for c in range(n_mxu, len(chunks)):
            o, n = offs[c], chunks[c]
            gc = gt[o - (F - nv):o - (F - nv) + n, :]
            gc = jnp.concatenate([gc] * (D // 128), axis=1)
            wait_all(w4buf.at[pl.ds(o, n), :], tsem.at[2 + c])
            prod = w4buf[pl.ds(o, n), :].astype(f32) * gc
            part = part + jnp.sum(prod.reshape(n // 8, 8, D), axis=0)

        y = y[0:1, :] + jnp.sum(part, axis=0, keepdims=True)
        o_ref[...] = y.astype(o_ref.dtype)

    kt = jnp.swapaxes(A_k_cache, 2, 3).reshape(H * DH, SK)
    vt = jnp.swapaxes(A_v_cache, 2, 3).reshape(H * DH, SK)
    out = pl.pallas_call(
        kernel,
        out_shape=jax.ShapeDtypeStruct((1, D), A_x.dtype),
        in_specs=[pl.BlockSpec(memory_space=pl.ANY)] * 7,
        out_specs=pl.BlockSpec(memory_space=pltpu.VMEM),
        scratch_shapes=[
            pltpu.VMEM((1, D), A_x.dtype),
            pltpu.VMEM((NBUF, D, R), A_wq.dtype),
            pltpu.VMEM((NBUF, R, W), A_k_cache.dtype),
            pltpu.VMEM((NBUF, R, W), A_v_cache.dtype),
            pltpu.VMEM((NBUF, R, D), A_wo.dtype),
            pltpu.VMEM((D, F), B_w3.dtype),
            pltpu.VMEM((F, D), B_w4.dtype),
            pltpu.SemaphoreType.DMA((4, NBUF)),
            pltpu.SemaphoreType.DMA((2 + len(chunks),)),
        ],
        compiler_params=pltpu.CompilerParams(
            vmem_limit_bytes=64 * 1024 * 1024,
            disable_semaphore_checks=True,
        ),
    )(A_x.reshape(1, D), kt, vt, A_wq, A_wo, B_w3, B_w4)
    return out.reshape(B, Sq, D)
```

```python
import functools

import jax
import jax.numpy as jnp
import numpy as np
from jax import lax
import jax.experimental.pallas as pl
import jax.experimental.pallas.tpu as pltpu

_EPS = 1e-5
_G = 2
_NBUF = 3
_M = 8
_AHEAD = 80
_PARTS = 4
_KV_TILE = (192, 128)
_WQ_TILE = (128, 128)
_WO_ROWS = 24
_W3_TILE = (64, 256)
_W4_ROWS = 32
_W4_MXU = (1024, 384)
_W4_VPU = (96, 32)


def _ln(x):
    m = jnp.mean(x, axis=-1, keepdims=True)
    d = x - m
    v = jnp.mean(d * d, axis=-1, keepdims=True)
    return d / jnp.sqrt(v + _EPS)


def _gelu(x):
    c = float(np.sqrt(2.0 / np.pi))
    return 0.5 * x * (1.0 + jnp.tanh(c * (x + 0.044715 * (x * x * x))))


def _tiles(rows, cols, tr, tc, row_major=True):
    assert rows % tr == 0 and cols % tc == 0
    if row_major:
        return [(r, c) for r in range(0, rows, tr) for c in range(0, cols, tc)]
    return [(r, c) for c in range(0, cols, tc) for r in range(0, rows, tr)]


@jax.jit
def pallas_sequential_preLN__sliding_block_cached__mixer_s_mlp__decode_kernel(
    A_x: jax.Array,
    A_k_cache: jax.Array,
    A_v_cache: jax.Array,
    A_wq: jax.Array,
    A_wo: jax.Array,
    B_x: jax.Array,
    B_w1: jax.Array,
    B_w2: jax.Array,
    B_w3: jax.Array,
    B_w4: jax.Array,
):
    B, Sq, D = A_x.shape
    _, H, SK, DH = A_k_cache.shape
    F = B_w3.shape[1]
    assert B == 1 and Sq == 1 and A_wq.shape == (D, H * DH) and H % _G == 0
    W = min(4096, max(256, SK // 4))
    G, NBUF, M = _G, _NBUF, _M
    R = G * DH
    nblk = H // G
    scale = float(DH ** -0.5)
    f32, bf16 = jnp.float32, jnp.bfloat16

    chunks = _W4_MXU + _W4_VPU
    offs = tuple(sum(chunks[:c]) for c in range(len(chunks)))
    n_mxu, nv = len(_W4_MXU), sum(_W4_VPU)
    assert sum(chunks) == F and nblk >= 2 and nv % 128 == 0 and D % 128 == 0
    assert R % _WO_ROWS == 0 and all(n % _W4_ROWS == 0 for n in chunks)

    def kernel(x_hbm, k_hbm, v_hbm, wq_hbm, wo_hbm, w3_hbm, w4_hbm, o_ref,
               xbuf, wqbuf, kbuf, vbuf, wobuf, w3buf, w4buf, sems, tsem):
        copy = pltpu.make_async_copy
        lazy = functools.partial

        def stage_stream(g, slot):
            kr, kc = _KV_TILE
            kv = []
            for r, c in _tiles(R, W, kr, kc):
                src = (pl.ds(g * R + r, kr), pl.ds(SK - W + c, kc))
                dst = (slot, pl.ds(r, kr), pl.ds(c, kc))
                kv.append(lazy(copy, k_hbm.at[src], kbuf.at[dst], sems.at[0, slot]))
                kv.append(lazy(copy, v_hbm.at[src], vbuf.at[dst], sems.at[1, slot]))
            qr, qc = _WQ_TILE
            wq = [lazy(copy, wq_hbm.at[pl.ds(r, qr), pl.ds(g * R + c, qc)],
                       wqbuf.at[slot, pl.ds(r, qr), pl.ds(c, qc)], sems.at[2, slot])
                  for r, c in _tiles(D, R, qr, qc, row_major=False)]
            wo = [lazy(copy, wo_hbm.at[pl.ds(g * R + r, _WO_ROWS), :],
                       wobuf.at[slot, pl.ds(r, _WO_ROWS), :], sems.at[3, slot])
                  for r in range(0, R, _WO_ROWS)]
            wts = [e for j in range(max(len(wq), len(wo))) for e in wq[j:j + 1] + wo[j:j + 1]]
            groups = (len(wts) + 1) // 2
            step = len(kv) // groups
            out = []
            for j in range(groups):
                out += kv[j * step:(j + 1) * step] + wts[2 * j:2 * j + 2]
            return out + kv[groups * step:]

        def tail_stream():
            tr, tc = _W3_TILE
            out = [lazy(copy, w3_hbm.at[pl.ds(r, tr), pl.ds(c, tc)],
                        w3buf.at[pl.ds(r, tr), pl.ds(c, tc)], tsem.at[1])
                   for r, c in _tiles(D, F, tr, tc)]
            for ci, (o, n) in enumerate(zip(offs, chunks)):
                out += [lazy(copy, w4_hbm.at[pl.ds(r, _W4_ROWS), :],
                             w4buf.at[pl.ds(r, _W4_ROWS), :], tsem.at[2 + ci])
                        for r in range(o, o + n, _W4_ROWS)]
            return out

        def start(stream, lo, hi, n_last=0):
            for i in range(lo, hi):
                stream[i]().start(priority=1 if i >= len(stream) - n_last else i % 2)

        def wait_all(buf, sem):
            copy(buf, buf, sem).wait()

        NE = len(stage_stream(0, 0))
        tail = tail_stream()
        NT = len(tail)
        O = _AHEAD
        n_vpu_copies = nv // _W4_ROWS
        assert O <= min(NE, NT)
        cut = [2 * ((NE * p) // (2 * _PARTS)) for p in range(_PARTS)] + [NE]
        tcut = [O + 2 * (((NT - O) * p) // (2 * _PARTS)) for p in range(_PARTS)] + [NT]

        def issue(g, part):
            lo, hi = cut[part], cut[part + 1]
            if lo < NE - O:
                @pl.when(g + 1 < nblk)
                def _():
                    start(stage_stream(g + 1, (g + 1) % NBUF), O + lo, O + min(hi, NE - O))
            if hi > NE - O:
                a, b = max(lo, NE - O) - (NE - O), hi - (NE - O)

                @pl.when(g + 2 < nblk)
                def _():
                    start(stage_stream(g + 2, (g + 2) % NBUF), a, b)

                @pl.when(g + 2 == nblk)
                def _():
                    start(tail, a, b, n_vpu_copies)
            if tcut[part] < tcut[part + 1]:
                @pl.when(g + 1 == nblk)
                def _():
                    start(tail, tcut[part], tcut[part + 1], n_vpu_copies)

        x_cp = copy(x_hbm, xbuf, tsem.at[0])
        first = stage_stream(0, 0)
        x_cp.start()
        start(first, 0, 16)
        x_cp.wait()
        start(first, 16, NE)
        start(stage_stream(1, 1), 0, O)

        x = jnp.broadcast_to(xbuf[...].astype(f32), (M, D))
        xn = _ln(x).astype(bf16)

        row = lax.broadcasted_iota(jnp.int32, (M, R), 0)
        col = lax.broadcasted_iota(jnp.int32, (M, R), 1)
        bd = (col >= row * DH) & (col < (row + 1) * DH)

        def stage(g, acc):
            slot = g % NBUF
            wait_all(kbuf.at[slot], sems.at[0, slot])
            wait_all(vbuf.at[slot], sems.at[1, slot])
            wait_all(wqbuf.at[slot], sems.at[2, slot])
            wait_all(wobuf.at[slot], sems.at[3, slot])

            issue(g, 0)
            q = jnp.dot(xn, wqbuf[slot], preferred_element_type=f32)
            qbd = jnp.where(bd, q, 0.0).astype(bf16)
            s = jnp.dot(qbd, kbuf[slot], preferred_element_type=f32)
            issue(g, 1)
            m = jnp.max(s, axis=-1, keepdims=True)
            p = jnp.exp((s - m) * scale)
            l = jnp.sum(p, axis=-1, keepdims=True)
            pb = p.astype(bf16)
            issue(g, 2)
            o = lax.dot_general(pb, vbuf[slot], (((1,), (1,)), ((), ())),
                                preferred_element_type=f32)
            for part in range(3, _PARTS):
                issue(g, part)
            obd = jnp.where(bd, o / l, 0.0).astype(bf16)
            return acc + jnp.dot(obd, wobuf[slot], preferred_element_type=f32)

        acc = lax.fori_loop(0, nblk, stage, jnp.zeros((M, D), f32))

        h = x + jnp.broadcast_to(jnp.sum(acc, axis=0, keepdims=True), (M, D))
        xb = _ln(h)
        xn2 = _ln(xb).astype(bf16)

        wait_all(w3buf, tsem.at[1])
        g1 = _gelu(jnp.dot(xn2, w3buf[...], preferred_element_type=f32)).astype(bf16)

        y = h + xb
        for c in range(n_mxu):
            o, n = offs[c], chunks[c]
            wait_all(w4buf.at[pl.ds(o, n), :], tsem.at[2 + c])
            y = y + jnp.dot(g1[:, o:o + n], w4buf[pl.ds(o, n), :],
                            preferred_element_type=f32)

        gt = jnp.concatenate(
            [jnp.concatenate([g1[:, o:o + 128].astype(f32)] * (128 // M), axis=0).T
             for o in range(F - nv, F, 128)], axis=0)
        part = jnp.zeros((8, D), f32)
        for c in range(n_mxu, len(chunks)):
            o, n = offs[c], chunks[c]
            gc = gt[o - (F - nv):o - (F - nv) + n, :]
            gc = jnp.concatenate([gc] * (D // 128), axis=1)
            wait_all(w4buf.at[pl.ds(o, n), :], tsem.at[2 + c])
            prod = w4buf[pl.ds(o, n), :].astype(f32) * gc
            part = part + jnp.sum(prod.reshape(n // 8, 8, D), axis=0)

        y = y[0:1, :] + jnp.sum(part, axis=0, keepdims=True)
        o_ref[...] = y.astype(o_ref.dtype)

    kt = jnp.swapaxes(A_k_cache, 2, 3).reshape(H * DH, SK)
    vt = jnp.swapaxes(A_v_cache, 2, 3).reshape(H * DH, SK)
    out = pl.pallas_call(
        kernel,
        out_shape=jax.ShapeDtypeStruct((1, D), A_x.dtype),
        in_specs=[pl.BlockSpec(memory_space=pl.ANY)] * 7,
        out_specs=pl.BlockSpec(memory_space=pltpu.VMEM),
        scratch_shapes=[
            pltpu.VMEM((1, D), A_x.dtype),
            pltpu.VMEM((NBUF, D, R), A_wq.dtype),
            pltpu.VMEM((NBUF, R, W), A_k_cache.dtype),
            pltpu.VMEM((NBUF, R, W), A_v_cache.dtype),
            pltpu.VMEM((NBUF, R, D), A_wo.dtype),
            pltpu.VMEM((D, F), B_w3.dtype),
            pltpu.VMEM((F, D), B_w4.dtype),
            pltpu.SemaphoreType.DMA((4, NBUF)),
            pltpu.SemaphoreType.DMA((2 + len(chunks),)),
        ],
        compiler_params=pltpu.CompilerParams(
            vmem_limit_bytes=64 * 1024 * 1024,
            disable_semaphore_checks=True,
        ),
    )(A_x.reshape(1, D), kt, vt, A_wq, A_wo, B_w3, B_w4)
    return out.reshape(B, Sq, D)
```

```python
import functools

import jax
import jax.numpy as jnp
import numpy as np
from jax import lax
import jax.experimental.pallas as pl
import jax.experimental.pallas.tpu as pltpu

_EPS = 1e-5
_G = 2
_NBUF = 3
_M = 8
_AHEAD = 80
_PARTS = 4
_K_TILE = (192, 128)
_V_TILE = (48, 512)
_WQ_TILE = (128, 128)
_WO_ROWS = 24
_W3_TILE = (64, 256)
_W4_ROWS = 32
_W4_STRIDE = (4, 2, 1, 1)
_W4_MXU = (1024, 384)
_W4_VPU = (96, 32)


def _ln(x):
    m = jnp.mean(x, axis=-1, keepdims=True)
    d = x - m
    v = jnp.mean(d * d, axis=-1, keepdims=True)
    return d / jnp.sqrt(v + _EPS)


def _gelu(x):
    c = float(np.sqrt(2.0 / np.pi))
    return 0.5 * x * (1.0 + jnp.tanh(c * (x + 0.044715 * (x * x * x))))


def _tiles(rows, cols, tr, tc, row_major=True):
    assert rows % tr == 0 and cols % tc == 0
    if row_major:
        return [(r, c) for r in range(0, rows, tr) for c in range(0, cols, tc)]
    return [(r, c) for c in range(0, cols, tc) for r in range(0, rows, tr)]


@jax.jit
def pallas_sequential_preLN__sliding_block_cached__mixer_s_mlp__decode_kernel(
    A_x: jax.Array,
    A_k_cache: jax.Array,
    A_v_cache: jax.Array,
    A_wq: jax.Array,
    A_wo: jax.Array,
    B_x: jax.Array,
    B_w1: jax.Array,
    B_w2: jax.Array,
    B_w3: jax.Array,
    B_w4: jax.Array,
):
    B, Sq, D = A_x.shape
    _, H, SK, DH = A_k_cache.shape
    F = B_w3.shape[1]
    assert B == 1 and Sq == 1 and A_wq.shape == (D, H * DH) and H % _G == 0
    W = min(4096, max(256, SK // 4))
    G, NBUF, M = _G, _NBUF, _M
    R = G * DH
    nblk = H // G
    scale = float(DH ** -0.5)
    f32, bf16 = jnp.float32, jnp.bfloat16

    chunks = _W4_MXU + _W4_VPU
    offs = tuple(sum(chunks[:c]) for c in range(len(chunks)))
    n_mxu, nv = len(_W4_MXU), sum(_W4_VPU)
    assert sum(chunks) == F and nblk >= 2 and nv % 128 == 0 and D % 128 == 0
    assert R % _WO_ROWS == 0 and all(n % _W4_ROWS == 0 for n in chunks)
    assert len(_W4_STRIDE) == len(chunks)

    def kernel(x_hbm, k_hbm, v_hbm, wq_hbm, wo_hbm, w3_hbm, w4_hbm, o_ref,
               xbuf, wqbuf, kbuf, vbuf, wobuf, w3buf, w4buf, sems, tsem):
        copy = pltpu.make_async_copy
        lazy = functools.partial

        def stage_stream(g, slot):
            def cache(hbm, buf, sem, tile, row_major):
                tr, tc = tile
                return [lazy(copy, hbm.at[pl.ds(g * R + r, tr), pl.ds(SK - W + c, tc)],
                             buf.at[slot, pl.ds(r, tr), pl.ds(c, tc)], sem)
                        for r, c in _tiles(R, W, tr, tc, row_major)]

            ks = cache(k_hbm, kbuf, sems.at[0, slot], _K_TILE, True)
            vs = cache(v_hbm, vbuf, sems.at[1, slot], _V_TILE, False)
            assert len(ks) == len(vs)
            kv = [e for pair in zip(ks, vs) for e in pair]
            qr, qc = _WQ_TILE
            wq = [lazy(copy, wq_hbm.at[pl.ds(r, qr), pl.ds(g * R + c, qc)],
                       wqbuf.at[slot, pl.ds(r, qr), pl.ds(c, qc)], sems.at[2, slot])
                  for r, c in _tiles(D, R, qr, qc, row_major=False)]
            wo = [lazy(copy, wo_hbm.at[pl.ds(g * R + r, _WO_ROWS), :],
                       wobuf.at[slot, pl.ds(r, _WO_ROWS), :], sems.at[3, slot])
                  for r in range(0, R, _WO_ROWS)]
            wts = [e for j in range(max(len(wq), len(wo))) for e in wq[j:j + 1] + wo[j:j + 1]]
            groups = (len(wts) + 1) // 2
            step = len(kv) // groups
            out = []
            for j in range(groups):
                out += kv[j * step:(j + 1) * step] + wts[2 * j:2 * j + 2]
            return out + kv[groups * step:]

        def tail_stream():
            tr, tc = _W3_TILE
            out = [lazy(copy, w3_hbm.at[pl.ds(r, tr), pl.ds(c, tc)],
                        w3buf.at[pl.ds(r, tr), pl.ds(c, tc)], tsem.at[1])
                   for r, c in _tiles(D, F, tr, tc, row_major=False)]
            for ci, (o, n) in enumerate(zip(offs, chunks)):
                rows = list(range(o, o + n, _W4_ROWS))
                per = len(rows) // _W4_STRIDE[ci]
                assert per * _W4_STRIDE[ci] == len(rows)
                rows = [rows[(j % _W4_STRIDE[ci]) * per + j // _W4_STRIDE[ci]]
                        for j in range(len(rows))]
                out += [lazy(copy, w4_hbm.at[pl.ds(r, _W4_ROWS), :],
                             w4buf.at[pl.ds(r, _W4_ROWS), :], tsem.at[2 + ci])
                        for r in rows]
            return out

        def start(stream, lo, hi, n_last=0):
            for i in range(lo, hi):
                stream[i]().start(priority=1 if i >= len(stream) - n_last else i % 2)

        def wait_all(buf, sem):
            copy(buf, buf, sem).wait()

        NE = len(stage_stream(0, 0))
        tail = tail_stream()
        NT = len(tail)
        O = _AHEAD
        n_vpu_copies = nv // _W4_ROWS
        assert O <= min(NE, NT)
        cut = [2 * ((NE * p) // (2 * _PARTS)) for p in range(_PARTS)] + [NE]
        tcut = [O + 2 * (((NT - O) * p) // (2 * _PARTS)) for p in range(_PARTS)] + [NT]

        def issue(g, part):
            lo, hi = cut[part], cut[part + 1]
            if lo < NE - O:
                @pl.when(g + 1 < nblk)
                def _():
                    start(stage_stream(g + 1, (g + 1) % NBUF), O + lo, O + min(hi, NE - O))
            if hi > NE - O:
                a, b = max(lo, NE - O) - (NE - O), hi - (NE - O)

                @pl.when(g + 2 < nblk)
                def _():
                    start(stage_stream(g + 2, (g + 2) % NBUF), a, b)

                @pl.when(g + 2 == nblk)
                def _():
                    start(tail, a, b, n_vpu_copies)
            if tcut[part] < tcut[part + 1]:
                @pl.when(g + 1 == nblk)
                def _():
                    start(tail, tcut[part], tcut[part + 1], n_vpu_copies)

        x_cp = copy(x_hbm, xbuf, tsem.at[0])
        first = stage_stream(0, 0)
        x_cp.start()
        start(first, 0, 16)
        x_cp.wait()
        start(first, 16, NE)
        start(stage_stream(1, 1), 0, O)

        x = jnp.broadcast_to(xbuf[...].astype(f32), (M, D))
        xn = _ln(x).astype(bf16)

        row = lax.broadcasted_iota(jnp.int32, (M, R), 0)
        col = lax.broadcasted_iota(jnp.int32, (M, R), 1)
        bd = (col >= row * DH) & (col < (row + 1) * DH)

        def stage(g, acc):
            slot = g % NBUF
            wait_all(kbuf.at[slot], sems.at[0, slot])
            wait_all(vbuf.at[slot], sems.at[1, slot])
            wait_all(wqbuf.at[slot], sems.at[2, slot])
            wait_all(wobuf.at[slot], sems.at[3, slot])

            issue(g, 0)
            q = jnp.dot(xn, wqbuf[slot], preferred_element_type=f32)
            qbd = jnp.where(bd, q, 0.0).astype(bf16)
            s = jnp.dot(qbd, kbuf[slot], preferred_element_type=f32)
            issue(g, 1)
            m = jnp.max(s, axis=-1, keepdims=True)
            p = jnp.exp((s - m) * scale)
            l = jnp.sum(p, axis=-1, keepdims=True)
            pb = p.astype(bf16)
            issue(g, 2)
            o = lax.dot_general(pb, vbuf[slot], (((1,), (1,)), ((), ())),
                                preferred_element_type=f32)
            for part in range(3, _PARTS):
                issue(g, part)
            obd = jnp.where(bd, o / l, 0.0).astype(bf16)
            return acc + jnp.dot(obd, wobuf[slot], preferred_element_type=f32)

        acc = lax.fori_loop(0, nblk, stage, jnp.zeros((M, D), f32))

        h = x + jnp.broadcast_to(jnp.sum(acc, axis=0, keepdims=True), (M, D))
        xb = _ln(h)
        xn2 = _ln(xb).astype(bf16)

        wait_all(w3buf, tsem.at[1])
        g1 = _gelu(jnp.dot(xn2, w3buf[...], preferred_element_type=f32)).astype(bf16)

        y = h + xb
        for c in range(n_mxu):
            o, n = offs[c], chunks[c]
            wait_all(w4buf.at[pl.ds(o, n), :], tsem.at[2 + c])
            y = y + jnp.dot(g1[:, o:o + n], w4buf[pl.ds(o, n), :],
                            preferred_element_type=f32)

        gt = jnp.concatenate(
            [jnp.concatenate([g1[:, o:o + 128].astype(f32)] * (128 // M), axis=0).T
             for o in range(F - nv, F, 128)], axis=0)
        part = jnp.zeros((8, D), f32)
        for c in range(n_mxu, len(chunks)):
            o, n = offs[c], chunks[c]
            gc = gt[o - (F - nv):o - (F - nv) + n, :]
            gc = jnp.concatenate([gc] * (D // 128), axis=1)
            wait_all(w4buf.at[pl.ds(o, n), :], tsem.at[2 + c])
            prod = w4buf[pl.ds(o, n), :].astype(f32) * gc
            part = part + jnp.sum(prod.reshape(n // 8, 8, D), axis=0)

        y = y[0:1, :] + jnp.sum(part, axis=0, keepdims=True)
        o_ref[...] = y.astype(o_ref.dtype)

    kt = jnp.swapaxes(A_k_cache, 2, 3).reshape(H * DH, SK)
    vt = jnp.swapaxes(A_v_cache, 2, 3).reshape(H * DH, SK)
    out = pl.pallas_call(
        kernel,
        out_shape=jax.ShapeDtypeStruct((1, D), A_x.dtype),
        in_specs=[pl.BlockSpec(memory_space=pl.ANY)] * 7,
        out_specs=pl.BlockSpec(memory_space=pltpu.VMEM),
        scratch_shapes=[
            pltpu.VMEM((1, D), A_x.dtype),
            pltpu.VMEM((NBUF, D, R), A_wq.dtype),
            pltpu.VMEM((NBUF, R, W), A_k_cache.dtype),
            pltpu.VMEM((NBUF, R, W), A_v_cache.dtype),
            pltpu.VMEM((NBUF, R, D), A_wo.dtype),
            pltpu.VMEM((D, F), B_w3.dtype),
            pltpu.VMEM((F, D), B_w4.dtype),
            pltpu.SemaphoreType.DMA((4, NBUF)),
            pltpu.SemaphoreType.DMA((2 + len(chunks),)),
        ],
        compiler_params=pltpu.CompilerParams(
            vmem_limit_bytes=64 * 1024 * 1024,
            disable_semaphore_checks=True,
        ),
    )(A_x.reshape(1, D), kt, vt, A_wq, A_wo, B_w3, B_w4)
    return out.reshape(B, Sq, D)
```

```python
import functools

import jax
import jax.numpy as jnp
import numpy as np
from jax import lax
import jax.experimental.pallas as pl
import jax.experimental.pallas.tpu as pltpu

_EPS = 1e-5
_G = 2
_NBUF = 3
_M = 8
_AHEAD = 100
_PARTS = 4
_K_TILE = (96, 128)
_V_TILE = (24, 512)
_WQ_TILE = (128, 128)
_WO_ROWS = 24
_W3_TILE = (64, 256)
_W4_ROWS = 32
_W4_STRIDE = (4, 2, 1, 1)
_W4_MXU = (1024, 384)
_W4_VPU = (96, 32)


def _ln(x):
    m = jnp.mean(x, axis=-1, keepdims=True)
    d = x - m
    v = jnp.mean(d * d, axis=-1, keepdims=True)
    return d / jnp.sqrt(v + _EPS)


def _gelu(x):
    c = float(np.sqrt(2.0 / np.pi))
    return 0.5 * x * (1.0 + jnp.tanh(c * (x + 0.044715 * (x * x * x))))


def _tiles(rows, cols, tr, tc, row_major=True):
    assert rows % tr == 0 and cols % tc == 0
    if row_major:
        return [(r, c) for r in range(0, rows, tr) for c in range(0, cols, tc)]
    return [(r, c) for c in range(0, cols, tc) for r in range(0, rows, tr)]


@jax.jit
def pallas_sequential_preLN__sliding_block_cached__mixer_s_mlp__decode_kernel(
    A_x: jax.Array,
    A_k_cache: jax.Array,
    A_v_cache: jax.Array,
    A_wq: jax.Array,
    A_wo: jax.Array,
    B_x: jax.Array,
    B_w1: jax.Array,
    B_w2: jax.Array,
    B_w3: jax.Array,
    B_w4: jax.Array,
):
    B, Sq, D = A_x.shape
    _, H, SK, DH = A_k_cache.shape
    F = B_w3.shape[1]
    assert B == 1 and Sq == 1 and A_wq.shape == (D, H * DH) and H % _G == 0
    W = min(4096, max(256, SK // 4))
    G, NBUF, M = _G, _NBUF, _M
    R = G * DH
    nblk = H // G
    scale = float(DH ** -0.5)
    f32, bf16 = jnp.float32, jnp.bfloat16

    chunks = _W4_MXU + _W4_VPU
    offs = tuple(sum(chunks[:c]) for c in range(len(chunks)))
    n_mxu, nv = len(_W4_MXU), sum(_W4_VPU)
    assert sum(chunks) == F and nblk >= 2 and nv % 128 == 0 and D % 128 == 0
    assert R % _WO_ROWS == 0 and all(n % _W4_ROWS == 0 for n in chunks)
    assert len(_W4_STRIDE) == len(chunks)

    def kernel(x_hbm, k_hbm, v_hbm, wq_hbm, wo_hbm, w3_hbm, w4_hbm, o_ref,
               xbuf, wqbuf, kbuf, vbuf, wobuf, w3buf, w4buf, sems, tsem):
        copy = pltpu.make_async_copy
        lazy = functools.partial

        def stage_stream(g, slot):
            def cache(hbm, buf, sem, tile, row_major):
                tr, tc = tile
                return [lazy(copy, hbm.at[pl.ds(g * R + r, tr), pl.ds(SK - W + c, tc)],
                             buf.at[slot, pl.ds(r, tr), pl.ds(c, tc)], sem)
                        for r, c in _tiles(R, W, tr, tc, row_major)]

            ks = cache(k_hbm, kbuf, sems.at[0, slot], _K_TILE, True)
            vs = cache(v_hbm, vbuf, sems.at[1, slot], _V_TILE, False)
            assert len(ks) == len(vs)
            kv = [e for pair in zip(ks, vs) for e in pair]
            qr, qc = _WQ_TILE
            wq = [lazy(copy, wq_hbm.at[pl.ds(r, qr), pl.ds(g * R + c, qc)],
                       wqbuf.at[slot, pl.ds(r, qr), pl.ds(c, qc)], sems.at[2, slot])
                  for r, c in _tiles(D, R, qr, qc, row_major=False)]
            wo = [lazy(copy, wo_hbm.at[pl.ds(g * R + r, _WO_ROWS), :],
                       wobuf.at[slot, pl.ds(r, _WO_ROWS), :], sems.at[3, slot])
                  for r in range(0, R, _WO_ROWS)]
            wts = [e for j in range(max(len(wq), len(wo))) for e in wq[j:j + 1] + wo[j:j + 1]]
            groups = (len(wts) + 1) // 2
            step = len(kv) // groups
            out = []
            for j in range(groups):
                out += kv[j * step:(j + 1) * step] + wts[2 * j:2 * j + 2]
            return out + kv[groups * step:]

        def tail_stream():
            tr, tc = _W3_TILE
            out = [lazy(copy, w3_hbm.at[pl.ds(r, tr), pl.ds(c, tc)],
                        w3buf.at[pl.ds(r, tr), pl.ds(c, tc)], tsem.at[1])
                   for r, c in _tiles(D, F, tr, tc, row_major=False)]
            for ci, (o, n) in enumerate(zip(offs, chunks)):
                rows = list(range(o, o + n, _W4_ROWS))
                per = len(rows) // _W4_STRIDE[ci]
                assert per * _W4_STRIDE[ci] == len(rows)
                rows = [rows[(j % _W4_STRIDE[ci]) * per + j // _W4_STRIDE[ci]]
                        for j in range(len(rows))]
                out += [lazy(copy, w4_hbm.at[pl.ds(r, _W4_ROWS), :],
                             w4buf.at[pl.ds(r, _W4_ROWS), :], tsem.at[2 + ci])
                        for r in rows]
            return out

        def start(stream, lo, hi, n_last=0):
            for i in range(lo, hi):
                stream[i]().start(priority=1 if i >= len(stream) - n_last else i % 2)

        def wait_all(buf, sem):
            copy(buf, buf, sem).wait()

        NE = len(stage_stream(0, 0))
        tail = tail_stream()
        NT = len(tail)
        O = _AHEAD
        n_vpu_copies = nv // _W4_ROWS
        assert O <= min(NE, NT)
        cut = [2 * ((NE * p) // (2 * _PARTS)) for p in range(_PARTS)] + [NE]
        tcut = [O + 2 * (((NT - O) * p) // (2 * _PARTS)) for p in range(_PARTS)] + [NT]

        def issue(g, part):
            lo, hi = cut[part], cut[part + 1]
            if lo < NE - O:
                @pl.when(g + 1 < nblk)
                def _():
                    start(stage_stream(g + 1, (g + 1) % NBUF), O + lo, O + min(hi, NE - O))
            if hi > NE - O:
                a, b = max(lo, NE - O) - (NE - O), hi - (NE - O)

                @pl.when(g + 2 < nblk)
                def _():
                    start(stage_stream(g + 2, (g + 2) % NBUF), a, b)

                @pl.when(g + 2 == nblk)
                def _():
                    start(tail, a, b, n_vpu_copies)
            if tcut[part] < tcut[part + 1]:
                @pl.when(g + 1 == nblk)
                def _():
                    start(tail, tcut[part], tcut[part + 1], n_vpu_copies)

        x_cp = copy(x_hbm, xbuf, tsem.at[0])
        first = stage_stream(0, 0)
        x_cp.start()
        start(first, 0, 64)
        x_cp.wait()
        start(first, 64, NE)
        start(stage_stream(1, 1), 0, O)

        x = jnp.broadcast_to(xbuf[...].astype(f32), (M, D))
        xn = _ln(x).astype(bf16)

        row = lax.broadcasted_iota(jnp.int32, (M, R), 0)
        col = lax.broadcasted_iota(jnp.int32, (M, R), 1)
        bd = (col >= row * DH) & (col < (row + 1) * DH)

        def stage(g, acc):
            slot = g % NBUF
            wait_all(kbuf.at[slot], sems.at[0, slot])
            wait_all(vbuf.at[slot], sems.at[1, slot])
            wait_all(wqbuf.at[slot], sems.at[2, slot])
            wait_all(wobuf.at[slot], sems.at[3, slot])

            issue(g, 0)
            q = jnp.dot(xn, wqbuf[slot], preferred_element_type=f32)
            qbd = jnp.where(bd, q, 0.0).astype(bf16)
            s = jnp.dot(qbd, kbuf[slot], preferred_element_type=f32)
            issue(g, 1)
            m = jnp.max(s, axis=-1, keepdims=True)
            p = jnp.exp((s - m) * scale)
            l = jnp.sum(p, axis=-1, keepdims=True)
            pb = p.astype(bf16)
            issue(g, 2)
            o = lax.dot_general(pb, vbuf[slot], (((1,), (1,)), ((), ())),
                                preferred_element_type=f32)
            for part in range(3, _PARTS):
                issue(g, part)
            obd = jnp.where(bd, o / l, 0.0).astype(bf16)
            return acc + jnp.dot(obd, wobuf[slot], preferred_element_type=f32)

        acc = lax.fori_loop(0, nblk, stage, jnp.zeros((M, D), f32))

        h = x + jnp.broadcast_to(jnp.sum(acc, axis=0, keepdims=True), (M, D))
        xb = _ln(h)
        xn2 = _ln(xb).astype(bf16)

        wait_all(w3buf, tsem.at[1])
        g1 = _gelu(jnp.dot(xn2, w3buf[...], preferred_element_type=f32)).astype(bf16)

        y = h + xb
        for c in range(n_mxu):
            o, n = offs[c], chunks[c]
            wait_all(w4buf.at[pl.ds(o, n), :], tsem.at[2 + c])
            y = y + jnp.dot(g1[:, o:o + n], w4buf[pl.ds(o, n), :],
                            preferred_element_type=f32)

        gt = jnp.concatenate(
            [jnp.concatenate([g1[:, o:o + 128].astype(f32)] * (128 // M), axis=0).T
             for o in range(F - nv, F, 128)], axis=0)
        part = jnp.zeros((8, D), f32)
        for c in range(n_mxu, len(chunks)):
            o, n = offs[c], chunks[c]
            gc = gt[o - (F - nv):o - (F - nv) + n, :]
            gc = jnp.concatenate([gc] * (D // 128), axis=1)
            wait_all(w4buf.at[pl.ds(o, n), :], tsem.at[2 + c])
            prod = w4buf[pl.ds(o, n), :].astype(f32) * gc
            part = part + jnp.sum(prod.reshape(n // 8, 8, D), axis=0)

        y = y[0:1, :] + jnp.sum(part, axis=0, keepdims=True)
        o_ref[...] = y.astype(o_ref.dtype)

    kt = jnp.swapaxes(A_k_cache, 2, 3).reshape(H * DH, SK)
    vt = jnp.swapaxes(A_v_cache, 2, 3).reshape(H * DH, SK)
    out = pl.pallas_call(
        kernel,
        out_shape=jax.ShapeDtypeStruct((1, D), A_x.dtype),
        in_specs=[pl.BlockSpec(memory_space=pl.ANY)] * 7,
        out_specs=pl.BlockSpec(memory_space=pltpu.VMEM),
        scratch_shapes=[
            pltpu.VMEM((1, D), A_x.dtype),
            pltpu.VMEM((NBUF, D, R), A_wq.dtype),
            pltpu.VMEM((NBUF, R, W), A_k_cache.dtype),
            pltpu.VMEM((NBUF, R, W), A_v_cache.dtype),
            pltpu.VMEM((NBUF, R, D), A_wo.dtype),
            pltpu.VMEM((D, F), B_w3.dtype),
            pltpu.VMEM((F, D), B_w4.dtype),
            pltpu.SemaphoreType.DMA((4, NBUF)),
            pltpu.SemaphoreType.DMA((2 + len(chunks),)),
        ],
        compiler_params=pltpu.CompilerParams(
            vmem_limit_bytes=64 * 1024 * 1024,
            disable_semaphore_checks=True,
        ),
    )(A_x.reshape(1, D), kt, vt, A_wq, A_wo, B_w3, B_w4)
    return out.reshape(B, Sq, D)
```
